```python
import os as _os
_os.environ.setdefault("JAX_PLATFORMS", "cpu")
import jax
import jax.numpy as jnp

def _softmax(x, axis=-1):
    return jax.nn.softmax(x, axis=axis)
def _gelu(x):
    return jax.nn.gelu(x, approximate=True)
def _silu(x):
    return jax.nn.silu(x)
def _sigmoid(x):
    return jax.nn.sigmoid(x)
def _layernorm(x, axis=-1, eps=1e-5):
    m = jnp.mean(x, axis=axis, keepdims=True)
    v = jnp.var(x, axis=axis, keepdims=True)
    return (x - m) / jnp.sqrt(v + eps)
def _scatter_add(tgt, idx, src, axis=0):
    return tgt.at[idx].add(src)
def _segment_sum(src, seg, n):
    return jax.ops.segment_sum(src, seg, n)
class _Rng:
    def __init__(self, key):
        self._k = key
    def _next(self):
        self._k, sub = jax.random.split(self._k)
        return sub
    def normal(self, shape):
        return jax.random.normal(self._next(), shape, dtype=jnp.bfloat16)
    def randint(self, lo, hi, shape):
        return jax.random.randint(self._next(), shape, lo, hi, dtype=jnp.int32)
    def uniform(self, shape, lo=0.0, hi=1.0):
        return jax.random.uniform(self._next(), shape, jnp.bfloat16, lo, hi)
    def permutation(self, n):
        return jax.random.permutation(self._next(), n)


kernel_name = 'gated_mix__mha_block__dense_activation_mish__prompt'

def setup_inputs():
    _rng = _Rng(jax.random.key(int.from_bytes(__import__("os").urandom(4), "little")))
    _w = (lambda a: (lambda t: t.astype(jnp.bfloat16) if jnp.issubdtype(t.dtype, jnp.floating) else t)(jnp.asarray(a)))
    def _A_setup():
        B, S, D, H = 1, 2048, 640, 32
        return {
            "x": _w((lambda *s: _rng.normal(s) * 0.05)(B, S, D)),
            "wqkv": _w((lambda *s: _rng.normal(s) * 0.2)(D, 3 * D)),
            "wo": _w((lambda *s: _rng.normal(s) * 0.05)(D, D)),
        }
    _A_in = _A_setup()

    def _B_setup():
        B, S, D, F = 1, 2048, 640, 1536
        return {
            "x": _w((lambda *s: _rng.normal(s) * 0.05)(B, S, D)),
            "w1": _w((lambda *s: _rng.normal(s) * 0.8)(D, F) * (D ** -0.5)),
            "b1": _w((lambda *s: _rng.normal(s) * 0.05)(F)),
            "w2": _w((lambda *s: _rng.normal(s) * 0.05)(F, D) * (F ** -0.5)),
        }
    _B_in = _B_setup()

    return {
        "A_x": _A_in["x"],
        "A_wqkv": _A_in["wqkv"],
        "A_wo": _A_in["wo"],
        "B_x": _B_in["x"],
        "B_w1": _B_in["w1"],
        "B_b1": _B_in["b1"],
        "B_w2": _B_in["w2"],
        "gate_w": _w((lambda *s: _rng.normal(s) * 0.05)(640) * 16.0),
    }

def reference(A_x, A_wqkv, A_wo, B_x, B_w1, B_b1, B_w2, gate_w):
    def _A_ref(x, wqkv, wo):
        B, S, D = x.shape
        H = 32
        Dh = D // H
        qkv = (lambda x, *d: x.transpose(*d))((x @ wqkv).reshape(B, S, 3, H, Dh), 2, 0, 3, 1, 4)
        q, k, v = qkv[0], qkv[1], qkv[2]
        scores = jnp.einsum("bhqd,bhkd->bhqk", q, k) * (Dh ** -0.5)
        p = _softmax(scores, axis=-1)
        o = jnp.einsum("bhqk,bhkd->bhqd", p, v)
        return (lambda x, *d: x.transpose(*d))(o, 0, 2, 1, 3).reshape(B, S, D) @ wo

    def _B_ref(x, w1, b1, w2):
        h = jnp.einsum("bsd,df->bsf", x, w1) + b1
        sp = jnp.log1p(jnp.exp(-jnp.abs(h))) + jnp.where(h > 0, h, jnp.zeros_like(h))
        act = h * jnp.tanh(sp)
        return jnp.einsum("bsf,fd->bsd", act, w2)

    x = A_x
    g = _sigmoid((x * gate_w).sum(-1, keepdims=True))
    a = _A_ref(x, A_wqkv, A_wo)
    b = _B_ref(x, B_w1, B_b1, B_w2)
    return g * a + (1 - g) * b
```

```python
import functools
import math

import jax
import jax.numpy as jnp
import jax.experimental.pallas as pl
import jax.experimental.pallas.tpu as pltpu
from jax import lax

_H = 32
_BQ = 512
_LANES = 128
_VROWS = 24

_NN = (((1,), (0,)), ((), ()))
_NT = (((1,), (1,)), ((), ()))
_TT = (((0,), (1,)), ((), ()))
_TN = (((0,), (0,)), ((), ()))


def _mm(a, b, dims=_NN):
    return lax.dot_general(a, b, dims, preferred_element_type=jnp.float32)


def _store_tiles(dst, val):
    nt = val.shape[1] // _LANES
    tiles = [val[:, j * _LANES:(j + 1) * _LANES] for j in range(nt)]
    lane = lax.broadcasted_iota(jnp.int32, tiles[0].shape, 1)
    for j in range(nt):
        dst[j] = tiles[j].astype(jnp.bfloat16)
    for j in range(nt - 1):
        dst[nt + j] = jnp.where(lane >= 64, tiles[j], tiles[j + 1]).astype(jnp.bfloat16)


def _kernel(x_ref, wqkv_ref, wo_ref, w1_ref, b1_ref, w2_ref, gw_ref, out_ref,
            kt, vt, qt, s_a, s_b, ot, *, d_model, dh):
    D = d_model
    S = x_ref.shape[0]
    nt = D // _LANES
    qi = pl.program_id(0)
    q0 = pl.multiple_of(qi * _BQ, _BQ)

    @pl.when(qi == 0)
    def _kv_setup():
        ck = 512
        for c in range(S // ck):
            rows = pl.ds(c * ck, ck)
            xc = x_ref[rows, :]
            k = _mm(xc, wqkv_ref[:, D:2 * D])
            tiles = [k[:, j * _LANES:(j + 1) * _LANES] for j in range(nt)]
            lane = lax.broadcasted_iota(jnp.int32, tiles[0].shape, 1)
            for j in range(nt):
                kt[j, rows, :] = tiles[j].astype(jnp.bfloat16)
            for j in range(nt - 1):
                kt[nt + j, rows, :] = jnp.where(lane >= 64, tiles[j], tiles[j + 1]).astype(jnp.bfloat16)
            v_t = _mm(wqkv_ref[:, 2 * D:3 * D], xc, _TT)
            v_t = v_t.astype(jnp.bfloat16).astype(jnp.float32)
            row = lax.broadcasted_iota(jnp.int32, (_VROWS - dh, ck), 0)
            tail = jnp.where(row == 0, 1.0, 0.0).astype(jnp.float32)
            for h in range(_H):
                vt[h, :, rows] = jnp.concatenate([v_t[h * dh:(h + 1) * dh, :], tail], axis=0)

    xq = x_ref[pl.ds(q0, _BQ), :]
    q = _mm(xq, wqkv_ref[:, 0:D]) * (dh ** -0.5 * math.log2(math.e))
    _store_tiles(qt, q)

    lane = lax.broadcasted_iota(jnp.int32, (16, _LANES), 1)

    def qk(h, sbuf):
        c0 = h * dh
        ja = c0 // _LANES
        jb = (c0 + dh - 1) // _LANES
        t = jnp.where(ja == jb, ja, nt + ja)
        base = jnp.where(jnp.logical_or(lane >= 64, ja == jb), ja, jb) * _LANES
        col = base + lane
        keep = jnp.logical_and(col >= c0, col < c0 + dh)
        qv = qt[t].reshape(_BQ // 16, 16, _LANES)
        qm = jnp.where(keep[None], qv, jnp.zeros_like(qv)).reshape(_BQ, _LANES)
        s = _mm(kt[t], qm, _NT)
        sbuf[...] = s
        return jnp.max(s, axis=0, keepdims=True)

    def smpv(h, sbuf, m):
        p = jnp.exp2(sbuf[...] - m).astype(jnp.bfloat16)
        o = _mm(vt[h], p)
        return o[:dh] * (1.0 / o[dh:dh + 1])

    def pair(g, m_a, last):
        m_b = qk(2 * g + 1, s_b)
        o_e = smpv(2 * g, s_a, m_a)
        m_n = None if last else qk(2 * g + 2, s_a)
        o_o = smpv(2 * g + 1, s_b, m_b)
        r0 = g * (2 * dh) if isinstance(g, int) else pl.multiple_of(g * (2 * dh), 8)
        ot[pl.ds(r0, 2 * dh), :] = jnp.concatenate([o_e, o_o], axis=0)
        return m_n

    m0 = qk(0, s_a)
    m_l = lax.fori_loop(0, _H // 2 - 1, lambda g, m: pair(g, m, False), m0)
    pair(_H // 2 - 1, m_l, True)

    a = _mm(ot[...].astype(jnp.bfloat16), wo_ref[...], _TN)

    F = w1_ref.shape[1]
    fc = 256
    b = jnp.zeros((_BQ, D), jnp.float32)
    for j in range(F // fc):
        cols = pl.ds(j * fc, fc)
        hh = _mm(xq, w1_ref[:, cols]) + b1_ref[:, cols].astype(jnp.float32)
        e = jnp.exp(jnp.minimum(hh, 20.0))
        n = e * (e + 2.0)
        act = hh * (n / (n + 2.0))
        b = b + _mm(act.astype(jnp.bfloat16), w2_ref[cols, :])

    z = jnp.sum(xq.astype(jnp.float32) * gw_ref[...].astype(jnp.float32), axis=-1, keepdims=True)
    g = 1.0 / (1.0 + jnp.exp(-z))
    out_ref[...] = (g * a + (1.0 - g) * b).astype(out_ref.dtype)


@jax.jit
def pallas_gated_mix__mha_block__dense_activation_mish__prompt_kernel(
    A_x: jax.Array,
    A_wqkv: jax.Array,
    A_wo: jax.Array,
    B_x: jax.Array,
    B_w1: jax.Array,
    B_b1: jax.Array,
    B_w2: jax.Array,
    gate_w: jax.Array,
):
    del B_x
    Bsz, S, D = A_x.shape
    assert Bsz == 1
    F = B_w1.shape[1]
    dh = D // _H
    nt = D // _LANES
    x = A_x.reshape(S, D)
    full = lambda shape: pl.BlockSpec(shape, lambda i: (0,) * len(shape))
    out = pl.pallas_call(
        functools.partial(_kernel, d_model=D, dh=dh),
        grid=(S // _BQ,),
        in_specs=[full((S, D)), full((D, 3 * D)), full((D, D)), full((D, F)), full((1, F)),
                  full((F, D)), full((1, D))],
        out_specs=pl.BlockSpec((_BQ, D), lambda i: (i, 0)),
        out_shape=jax.ShapeDtypeStruct((S, D), A_x.dtype),
        scratch_shapes=[
            pltpu.VMEM((2 * nt - 1, S, _LANES), jnp.bfloat16),
            pltpu.VMEM((_H, _VROWS, S), jnp.float32),
            pltpu.VMEM((2 * nt - 1, _BQ, _LANES), jnp.bfloat16),
            pltpu.VMEM((S, _BQ), jnp.float32),
            pltpu.VMEM((S, _BQ), jnp.float32),
            pltpu.VMEM((D, _BQ), jnp.float32),
        ],
        compiler_params=pltpu.CompilerParams(
            dimension_semantics=("arbitrary",), vmem_limit_bytes=100 * 2**20),
    )(x, A_wqkv, A_wo, B_w1, B_b1.reshape(1, F), B_w2, gate_w.reshape(1, D))
    return out.reshape(Bsz, S, D)
```

```python
import math

import jax
import jax.numpy as jnp
import jax.experimental.pallas as pl
import jax.experimental.pallas.tpu as pltpu
from jax import lax

_H = 32
_BQ = 512
_CK = 128
_U = 10
_RP = 128
_FB = 512
_LANES = 128
_VROWS = 24

_NN = (((1,), (0,)), ((), ()))
_NT = (((1,), (1,)), ((), ()))
_TT = (((0,), (1,)), ((), ()))
_TN = (((0,), (0,)), ((), ()))
_LOG2E = math.log2(math.e)


def _mm(a, b, dims=_NN):
    return lax.dot_general(a, b, dims, preferred_element_type=jnp.float32)


def _mish(h):
    e = jnp.exp2(jnp.minimum(h, 20.0) * _LOG2E)
    n = e * (e + 2.0)
    d = n + 2.0
    r = pltpu.reciprocal(d, approx=True)
    r = r * (2.0 - d * r)
    return h * (n * r)


def _kernel(x_hbm, wqkv_hbm, wo_hbm, w1_hbm, b1_ref, w2_hbm, gw_ref, out_hbm,
            x_v, wq_v, wk_v, wv_v, wo_v, w1_v, w2_v, sems,
            kt, vt, qm, s_a, s_b, ot, hpre, act, obuf, osems):
    S, D = x_v.shape
    F = w1_v.shape[1]
    dh = D // _H
    nt = D // _LANES
    nck = S // _CK
    qi = pl.program_id(0)
    q0 = pl.multiple_of(qi * _BQ, _BQ)

    @pl.when(qi == 0)
    def _kv_setup():
        ck = 512
        cps = {}

        def start(name, src, dst):
            cps[name] = pltpu.make_async_copy(src, dst, sems.at[len(cps)])
            cps[name].start()

        lane = lax.broadcasted_iota(jnp.int32, (ck, _LANES), 1)
        row = lax.broadcasted_iota(jnp.int32, (8, ck), 0)

        def keys_chunk(rows):
            k = _mm(x_v[rows, :], wk_v[...]).astype(jnp.bfloat16)
            tiles = [k[:, j * _LANES:(j + 1) * _LANES] for j in range(nt)]
            for j in range(nt):
                kt[j, rows, :] = tiles[j]
            for j in range(nt - 1):
                kt[nt + j, rows, :] = jnp.where(lane >= 64, tiles[j], tiles[j + 1])

        def values_chunk(rows):
            v_t = _mm(wv_v[...], x_v[rows, :], _TT)
            v_t = v_t.astype(jnp.bfloat16).astype(jnp.float32)
            for g in range(_H // 2):
                r = 2 * g * dh
                mid = v_t[r + 16:r + 24, :]
                vt[2 * g, 0:16, rows] = v_t[r:r + 16, :]
                vt[2 * g, 16:24, rows] = jnp.where(row < 4, mid, jnp.where(row == 4, 1.0, 0.0))
                vt[2 * g + 1, 0:8, rows] = jnp.where(row >= 4, mid, jnp.where(row == 0, 1.0, 0.0))
                vt[2 * g + 1, 8:24, rows] = v_t[r + 24:r + 40, :]

        start("wk", wqkv_hbm.at[:, pl.ds(D, D)], wk_v)
        start("x0", x_hbm.at[pl.ds(0, ck), :], x_v.at[pl.ds(0, ck), :])
        cps["wk"].wait()
        cps["x0"].wait()
        start("wv", wqkv_hbm.at[:, pl.ds(2 * D, D)], wv_v)
        start("x1", x_hbm.at[pl.ds(ck, S - ck), :], x_v.at[pl.ds(ck, S - ck), :])
        keys_chunk(pl.ds(0, ck))
        cps["wv"].wait()
        start("wq", wqkv_hbm.at[:, pl.ds(0, D)], wq_v)
        start("w1", w1_hbm, w1_v)
        start("wo", wo_hbm, wo_v)
        start("w2", w2_hbm, w2_v)
        values_chunk(pl.ds(0, ck))
        cps["x1"].wait()

        def chunk(c, carry):
            rows = pl.ds(pl.multiple_of(c * ck, ck), ck)
            values_chunk(rows)
            keys_chunk(rows)
            return carry

        lax.fori_loop(1, S // ck, chunk, 0)
        for name in ("wq", "w1", "wo", "w2"):
            cps[name].wait()

    def xq(r=None):
        if r is None:
            return x_v[pl.ds(q0, _BQ), :]
        return x_v[pl.ds(pl.multiple_of(q0 + r * _RP, _RP), _RP), :]

    b1 = b1_ref[...].astype(jnp.float32).reshape(1, F)

    def mlp1(r0, nr, j):
        cols = pl.ds(j * _FB, _FB)
        xs = x_v[pl.ds(pl.multiple_of(q0 + r0, nr), nr), :]
        hpre[pl.ds(r0, nr), cols] = _mm(xs, w1_v[:, cols]) + b1[:, j * _FB:(j + 1) * _FB]

    def activate(r, j):
        rows, cols = pl.ds(r * _RP, _RP), pl.ds(j * _FB, _FB)
        act[rows, cols] = _mish(hpre[rows, cols]).astype(jnp.bfloat16)

    def key_tile(h):
        c0 = h * dh
        ja = c0 // _LANES
        jb = (c0 + dh - 1) // _LANES
        return jnp.where(ja == jb, ja, nt + ja)

    bufs = (s_a, s_b)

    def pv(h, par, c, m):
        keys = pl.ds(c * _CK, _CK)
        p = jnp.exp2(bufs[par][keys, :] - m).astype(jnp.bfloat16)
        return _mm(vt[h, :, keys], p)

    def finalize(h, par, o):
        row = lax.broadcasted_iota(jnp.int32, (8, _BQ), 0)
        if par == 0:
            r0 = h * dh
            r0 = r0 if isinstance(r0, int) else pl.multiple_of(r0, 8)
            ot[pl.ds(r0, _VROWS), :] = o * (1.0 / o[dh:dh + 1])
        else:
            r0 = h * dh - 4
            r0 = r0 if isinstance(r0, int) else pl.multiple_of(r0, 8)
            o = o * (1.0 / o[0:1])
            ot[pl.ds(r0, 8), :] = jnp.where(row < 4, ot[pl.ds(r0, 8), :], o[0:8])
            ot[pl.ds(r0 + 8, 16), :] = o[8:24]

    def step(h, par, state, do_qk=True, do_pv=True, do_tail=True, extra=None, pre=None):
        m_prev, o_prev, m_cur = state
        m_new = None
        o = None
        if do_qk:
            t = key_tile(h + 1)
        for c in range(nck):
            if pre is not None:
                pre(c)
            if do_qk:
                keys = pl.ds(c * _CK, _CK)
                s = _mm(kt[t, keys, :], qm[h + 1])
                bufs[1 - par][keys, :] = s
                mc = jnp.max(s.reshape(_CK // 8, 8, _BQ), axis=0)
                m_new = mc if m_new is None else jnp.maximum(m_new, mc)
            if c == 0:
                if do_tail:
                    finalize(h - 1, 1 - par, o_prev + pv(h - 1, 1 - par, nck - 1, m_prev))
            elif do_pv:
                oc = pv(h, par, c - 1, m_cur)
                o = oc if o is None else o + oc
            if extra is not None:
                extra(c)
        if do_qk:
            m_new = jnp.max(m_new, axis=0, keepdims=True)
        return m_cur, o, m_new

    npc = _BQ // _RP
    for r in range(1):
        mlp1(r * _RP, _RP, 0)
    q_t = _mm(wq_v[...], xq(), _TT) * (dh ** -0.5 * _LOG2E)
    for r in range(1, npc):
        mlp1(r * _RP, _RP, 0)
    row = lax.broadcasted_iota(jnp.int32, (_LANES, _BQ), 0)
    for h in range(_H):
        c0 = h * dh
        ja = c0 // _LANES
        jb = (c0 + dh - 1) // _LANES
        if ja == jb:
            col = ja * _LANES + row
            tile = q_t[ja * _LANES:(ja + 1) * _LANES]
        else:
            col = jnp.where(row >= 64, ja, jb) * _LANES + row
            tile = jnp.concatenate([q_t[jb * _LANES:jb * _LANES + 64],
                                    q_t[ja * _LANES + 64:(ja + 1) * _LANES]], axis=0)
        keep = jnp.logical_and(col >= c0, col < c0 + dh)
        qm[h] = jnp.where(keep, tile, 0.0).astype(jnp.bfloat16)

    def mish_piece(c):
        if c % 4 == 0:
            activate(c // 4, 0)

    dummy = jnp.zeros((1, _BQ), jnp.float32)
    st = step(-1, 1, (dummy, None, dummy), do_pv=False, do_tail=False, extra=mish_piece)
    st = step(0, 0, st, do_tail=False)
    ng = (_H - 2) // _U

    def group(g, st):
        for u in range(_U):
            st = step(1 + g * _U + u, (1 + u) % 2, st)
        return st

    st = lax.fori_loop(0, ng, group, st)
    for h in range(1 + ng * _U, _H - 1):
        st = step(h, h % 2, st)

    def out_copy(blk, r):
        rows = pl.ds(r * _RP, _RP)
        dst = pl.ds(pl.multiple_of(blk * _BQ + r * _RP, _RP), _RP)
        return pltpu.make_async_copy(obuf.at[rows, :], out_hbm.at[dst, :], osems.at[r])

    @pl.when(qi > 0)
    def _drain_previous():
        for r in range(npc):
            out_copy(qi - 1, r).wait()

    def mlp_piece(c):
        mlp1(c * (_BQ // nck), _BQ // nck, 1)

    m_last, o_last, _ = step(_H - 1, (_H - 1) % 2, st, do_qk=False, pre=mlp_piece)
    finalize(_H - 1, (_H - 1) % 2, o_last + pv(_H - 1, (_H - 1) % 2, nck - 1, m_last))
    for r in range(npc):
        mlp1(r * _RP, _RP, 2)
        activate(r, 1)

    gw = gw_ref[...].astype(jnp.float32).reshape(1, D)
    for r in range(npc):
        rows = pl.ds(r * _RP, _RP)
        a = _mm(ot[:, rows].astype(jnp.bfloat16), wo_v[...], _TN)
        activate(r, 2)
        b = _mm(act[rows, :], w2_v[...])
        z = jnp.sum(xq(r).astype(jnp.float32) * gw, axis=-1, keepdims=True)
        g = 1.0 / (1.0 + jnp.exp(-z))
        obuf[rows, :] = (g * a + (1.0 - g) * b).astype(obuf.dtype)
        out_copy(qi, r).start()

    @pl.when(qi == pl.num_programs(0) - 1)
    def _drain_last():
        for r in range(npc):
            out_copy(qi, r).wait()


@jax.jit
def pallas_gated_mix__mha_block__dense_activation_mish__prompt_kernel(
    A_x: jax.Array,
    A_wqkv: jax.Array,
    A_wo: jax.Array,
    B_x: jax.Array,
    B_w1: jax.Array,
    B_b1: jax.Array,
    B_w2: jax.Array,
    gate_w: jax.Array,
):
    del B_x
    Bsz, S, D = A_x.shape
    assert (Bsz, S, D) == (1, 2048, 640) and B_w1.shape[1] == 3 * _FB
    F = B_w1.shape[1]
    nt = D // _LANES
    x = A_x.reshape(S, D)
    bf = jnp.bfloat16
    hbm = pl.BlockSpec(memory_space=pl.ANY)
    full = lambda shape: pl.BlockSpec(shape, lambda i: (0,) * len(shape))
    out = pl.pallas_call(
        _kernel,
        grid=(S // _BQ,),
        in_specs=[hbm, hbm, hbm, hbm, full((F,)), hbm, full((D,))],
        out_specs=hbm,
        out_shape=jax.ShapeDtypeStruct((S, D), A_x.dtype),
        scratch_shapes=[
            pltpu.VMEM((S, D), bf), pltpu.VMEM((D, D), bf), pltpu.VMEM((D, D), bf),
            pltpu.VMEM((D, D), bf), pltpu.VMEM((D, D), bf), pltpu.VMEM((D, F), bf),
            pltpu.VMEM((F, D), bf), pltpu.SemaphoreType.DMA((8,)),
            pltpu.VMEM((2 * nt - 1, S, _LANES), bf),
            pltpu.VMEM((_H, _VROWS, S), jnp.float32),
            pltpu.VMEM((_H, _LANES, _BQ), bf),
            pltpu.VMEM((S, _BQ), jnp.float32),
            pltpu.VMEM((S, _BQ), jnp.float32),
            pltpu.VMEM((D, _BQ), jnp.float32),
            pltpu.VMEM((_BQ, F), jnp.float32),
            pltpu.VMEM((_BQ, F), bf),
            pltpu.VMEM((_BQ, D), bf),
            pltpu.SemaphoreType.DMA((_BQ // _RP,)),
        ],
        compiler_params=pltpu.CompilerParams(
            dimension_semantics=("arbitrary",), vmem_limit_bytes=100 * 2**20),
    )(x, A_wqkv, A_wo, B_w1, B_b1, B_w2, gate_w)
    return out.reshape(Bsz, S, D)
```
